```python
import os as _os
_os.environ.setdefault('JAX_PLATFORMS', 'cpu')
import jax
import jax.numpy as jnp

def _softmax(x, axis=-1):
    return jax.nn.softmax(x, axis=axis)

def _gelu(x):
    return jax.nn.gelu(x, approximate=True)

def _silu(x):
    return jax.nn.silu(x)

def _sigmoid(x):
    return jax.nn.sigmoid(x)

def _layernorm(x, axis=-1, eps=1e-05):
    m = jnp.mean(x, axis=axis, keepdims=True)
    v = jnp.var(x, axis=axis, keepdims=True)
    return (x - m) / jnp.sqrt(v + eps)

def _scatter_add(tgt, idx, src, axis=0):
    return tgt.at[idx].add(src)

def _segment_sum(src, seg, n):
    return jax.ops.segment_sum(src, seg, n)

class _Rng:

    def __init__(self, key):
        self._k = key

    def _next(self):
        self._k, sub = jax.random.split(self._k)
        return sub

    def normal(self, shape):
        return jax.random.normal(self._next(), shape, dtype=jnp.bfloat16)

    def randint(self, lo, hi, shape):
        return jax.random.randint(self._next(), shape, lo, hi, dtype=jnp.int32)

    def uniform(self, shape, lo=0.0, hi=1.0):
        return jax.random.uniform(self._next(), shape, jnp.bfloat16, lo, hi)

    def permutation(self, n):
        return jax.random.permutation(self._next(), n)
kernel_name = 'parallel_sum__memory_aug_recurrent_mem_tr__dense_activation_gelu__prompt'

def setup_inputs():
    _rng = _Rng(jax.random.key(int.from_bytes(__import__("os").urandom(4), "little")))
    _w = lambda a: (lambda t: t.astype(jnp.bfloat16) if jnp.issubdtype(t.dtype, jnp.floating) else t)(jnp.asarray(a))

    def _A_setup():
        B, S, Dm = (1, 2048, 1024)
        H, Dh = (32, 128)
        M, seg = (8, 32)
        seg = min(seg, S)
        S = S // seg * seg
        return {'x': _w((lambda *s: _rng.normal(s) * 0.05)(B, S, Dm)), 'mem0': _w((lambda *s: _rng.normal(s) * 0.2)(B, M, Dm)), 'Wq': _w((lambda *s: _rng.normal(s) * 0.8)(Dm, H, Dh) * Dm ** (-0.5)), 'Wk': _w((lambda *s: _rng.normal(s) * 0.8)(Dm, H, Dh) * Dm ** (-0.5)), 'Wv': _w((lambda *s: _rng.normal(s) * 0.2)(Dm, H, Dh) * Dm ** (-0.5)), 'Wo': _w((lambda *s: _rng.normal(s) * 0.2)(H, Dh, Dm) * (H * Dh) ** (-0.5)), 'seg_len': seg}
    _A_in = _A_setup()

    def _B_setup():
        B, S, D, F = (1, 2048, 1024, 3584)
        return {'x': _w((lambda *s: _rng.normal(s) * 0.05)(B, S, D)), 'w1': _w((lambda *s: _rng.normal(s) * 0.1)(D, F) * D ** (-0.5)), 'b1': _w((lambda *s: _rng.normal(s) * 0.1)(F) * 0.01), 'w2': _w((lambda *s: _rng.normal(s) * 0.1)(F, D) * F ** (-0.5)), 'b2': _w((lambda *s: _rng.normal(s) * 0.05)(D) * 0.01)}
    _B_in = _B_setup()
    return {'A_x': _A_in['x'], 'A_mem0': _A_in['mem0'], 'A_Wq': _A_in['Wq'], 'A_Wk': _A_in['Wk'], 'A_Wv': _A_in['Wv'], 'A_Wo': _A_in['Wo'], 'A_seg_len': _A_in['seg_len'], 'B_x': _B_in['x'], 'B_w1': _B_in['w1'], 'B_b1': _B_in['b1'], 'B_w2': _B_in['w2'], 'B_b2': _B_in['b2']}

def reference(A_x, A_mem0, A_Wq, A_Wk, A_Wv, A_Wo, A_seg_len, B_x, B_w1, B_b1, B_w2, B_b2):

    def _A_ref(x, mem0, Wq, Wk, Wv, Wo, seg_len):
        B, S, Dm = x.shape
        H, Dh = (Wq.shape[1], Wq.shape[2])
        M = mem0.shape[1]
        scale = Dh ** (-0.5)
        n_seg = S // seg_len
        L = M + seg_len
        idx = jnp.arange(L)
        mask = (idx[:, None] < M) | (idx[:, None] >= idx[None, :])
        mem = mem0
        outs = []
        for s in range(n_seg):
            xs = x[:, s * seg_len:(s + 1) * seg_len, :].copy()
            h = jnp.concatenate([mem, xs], axis=1)
            q = jnp.einsum('btd,dhe->bhte', h, Wq)
            k = jnp.einsum('btd,dhe->bhte', h, Wk)
            v = jnp.einsum('btd,dhe->bhte', h, Wv)
            scores = jnp.einsum('bhqe,bhke->bhqk', q, k) * scale
            scores = jnp.where(mask[None, None], scores, -1000000000.0)
            p = _softmax(scores, axis=-1)
            o = jnp.einsum('bhqk,bhke->bhqe', p, v)
            o = jnp.einsum('bhte,hed->btd', o, Wo)
            mem = o[:, :M, :].copy()
            outs.append(o[:, M:, :])
        return jnp.concatenate(outs, axis=1)

    def _B_ref(x, w1, b1, w2, b2):
        h = jnp.einsum('bsd,df->bsf', x, w1) + b1
        h = _gelu(h)
        return jnp.einsum('bsf,fd->bsd', h, w2) + b2
    x = A_x
    xn = _layernorm(x, axis=-1)
    return x + _A_ref(xn, A_mem0, A_Wq, A_Wk, A_Wv, A_Wo, A_seg_len) + _B_ref(xn, B_w1, B_b1, B_w2, B_b2)
```

```python
import functools
import jax
import jax.numpy as jnp
from jax import lax
from jax.experimental import pallas as pl
from jax.experimental.pallas import tpu as pltpu

F32 = jnp.float32
BF16 = jnp.bfloat16
U32 = jnp.uint32

NT = (((1,), (1,)), ((), ()))
NN = (((1,), (0,)), ((), ()))

PVD = 1
UNR = 1
P2POS = 'c'
SCOPES = 0


def _dot(a, b, dims=NN):
    return lax.dot_general(a, b, dims, preferred_element_type=F32)


def _gelu_tanh(x):
    c = 0.7978845608028654
    return 0.5 * x * (1.0 + jnp.tanh(c * (x + 0.044715 * (x * x * x))))


def _tr8(vs, sub):
    vs = list(vs)
    for dist in (4, 2, 1):
        m = (sub & dist) == 0
        new = list(vs)
        for a in range(8):
            if a & dist:
                continue
            b = a + dist
            new[a] = jnp.where(m, vs[a], pltpu.roll(vs[b], dist, 0))
            new[b] = jnp.where(m, pltpu.roll(vs[a], 8 - dist, 0), vs[b])
        vs = new
    return vs


class _NoScope:
    def __enter__(self):
        return None

    def __exit__(self, *a):
        return False


def _scope(name):
    return jax.named_scope(name) if SCOPES else _NoScope()


def build(S, D, H, E, FF, MEM, SEG):
    L = MEM + SEG
    NSEG = S // SEG
    DB = D // 128
    FB = FF // 128
    XCH = 8
    XR = S // XCH
    P1C = 2
    P1N = FB // P1C
    P1R = 256
    RCH = 4
    RD = D // RCH
    scale = float(E) ** -0.5

    def kernel(x_hbm, mem0_ref, wq_hbm, wk_hbm, wv_hbm, wo_hbm, w1_hbm, b1_ref, w2_hbm, b2_ref,
               out_hbm,
               x_v, xn_v, h_v, out_v, stg, wqkv, wo_v, w1_v, w2_v, o_buf, b1f, b2f,
               sem_x, sem_w1, sem_w2, sem_wo, sem_stg, sem_out):
        w_hbm = (wq_hbm, wk_hbm, wv_hbm)

        def x_cp(c):
            return pltpu.make_async_copy(x_hbm.at[pl.ds(c * XR, XR), :], x_v.at[pl.ds(c * XR, XR), :], sem_x.at[c])

        def w1_cp(c):
            return pltpu.make_async_copy(w1_hbm.at[:, pl.ds(pl.multiple_of(c * 128, 128), 128)], w1_v.at[c], sem_w1.at[c])

        def w2_cp(c):
            return pltpu.make_async_copy(w2_hbm.at[:, pl.ds(c * 128, 128)], w2_v.at[c], sem_w2.at[c])

        def wo_cp(c):
            return pltpu.make_async_copy(wo_hbm.at[:, pl.ds(c * 128, 128)], wo_v.at[c], sem_wo.at[c])

        def stg_cp(t, c):
            return pltpu.make_async_copy(w_hbm[t].at[pl.ds(c * RD, RD)], stg.at[t, pl.ds(c * RD, RD)],
                                         sem_stg.at[t * RCH + c])

        x_cp(0).start()
        x_cp(1).start()
        b1f[...] = b1_ref[...].astype(F32)
        b2f[...] = b2_ref[...].astype(F32)

        def ln_rows(i, carry):
            r0 = pl.multiple_of(i * 64, 64)
            xb = x_v[pl.ds(r0, 64), :].astype(F32)
            m = jnp.mean(xb, axis=-1, keepdims=True)
            xc = xb - m
            v = jnp.mean(xc * xc, axis=-1, keepdims=True)
            xn_v[pl.ds(r0, 64), :] = xc * lax.rsqrt(v + 1e-5)
            return carry

        with _scope('LN'):
            for c in range(XCH):
                x_cp(c).wait()
                if c + 2 < XCH:
                    x_cp(c + 2).start()
                elif c + 2 == XCH:
                    for j in range(P1C):
                        w1_cp(j).start()
                else:
                    for j in range(P1C, 2 * P1C):
                        w1_cp(j).start()
                lax.fori_loop(c * (XR // 64), (c + 1) * (XR // 64), ln_rows, 0)

        w1u = w1_v.bitcast(U32)
        hu = h_v.bitcast(U32)

        def p1(it, carry):
            @pl.when(it + 2 < P1N)
            def _():
                for j in range(P1C):
                    w1_cp((it + 2) * P1C + j).start()
            for k in range(3 * RCH):
                @pl.when(it == k)
                def _(k=k):
                    stg_cp(k // RCH, k % RCH).start()
            @pl.when(it == 0)
            def _():
                for c in range(DB):
                    wo_cp(c).start()
            @pl.when(it == 4)
            def _():
                for c in range(DB):
                    w2_cp(c).start()
            for j in range(P1C):
                w1_cp(it * P1C + j).wait()
            for j in range(P1C):
                c = it * P1C + j
                w = pltpu.bitcast(w1u[c], BF16)
                b = b1f[pl.ds(c, 1), :]
                for r in range(S // P1R):
                    hh = _dot(xn_v[pl.ds(r * P1R, P1R), :], w) + b
                    hu[c, pl.ds(r * P1R // 2, P1R // 2), :] = pltpu.bitcast(_gelu_tanh(hh).astype(BF16), U32)
            return carry

        with _scope('P1'):
            lax.fori_loop(0, P1N, p1, 0)

        sub = lax.broadcasted_iota(jnp.int32, (8, 128), 0)
        stg_u = stg.bitcast(U32)
        wqkv_u = wqkv.bitcast(U32)
        with _scope('RL'):
            for t in range(3):
                for c in range(RCH):
                    stg_cp(t, c).wait()

                def rl(i, carry, t=t):
                    d0 = pl.multiple_of(i * 16, 16)
                    o0 = pl.multiple_of(i * 8, 8)
                    for half in range(H // 16):
                        Ev = _tr8([stg_u[t, d0 + 2 * j, pl.ds(half * 8, 8), :] for j in range(8)], sub)
                        Ov = _tr8([stg_u[t, d0 + 2 * j + 1, pl.ds(half * 8, 8), :] for j in range(8)], sub)
                        for s in range(8):
                            hp = half * 8 + s
                            lo = (Ev[s] & U32(0xFFFF)) | (Ov[s] << 16)
                            hi = (Ev[s] >> 16) | (Ov[s] & U32(0xFFFF0000))
                            wqkv_u[3 * (2 * hp) + t, pl.ds(o0, 8), :] = lo
                            wqkv_u[3 * (2 * hp + 1) + t, pl.ds(o0, 8), :] = hi
                    return carry
                lax.fori_loop(0, D // 16, rl, 0)

            for c in range(DB):
                wo_cp(c).wait()
                w2_cp(c).wait()

        wou = wo_v.bitcast(U32)
        w2u = w2_v.bitcast(U32)
        qi = lax.broadcasted_iota(jnp.int32, (L, L), 0)
        ki = lax.broadcasted_iota(jnp.int32, (L, L), 1)
        mask = (qi < MEM) | (qi >= ki)

        def out_cp(s):
            r0 = pl.multiple_of(s * SEG, SEG)
            return pltpu.make_async_copy(out_v.at[pl.ds(r0, SEG), :], out_hbm.at[pl.ds(r0, SEG), :], sem_out)

        def step(s, mem):
            r0 = pl.multiple_of(s * SEG, SEG)
            rh = pl.multiple_of(s * (SEG // 2), SEG // 2)
            lhs = jnp.concatenate([mem, xn_v[pl.ds(r0, SEG), :]], axis=0)
            W = lambda i: pltpu.bitcast(wqkv_u[i], BF16)
            qs, ks, vs_, es, ls, ys = {}, {}, {}, {}, {}, {}

            def do_y(nb):
                hrow = jnp.concatenate([pltpu.bitcast(hu[kc, pl.ds(rh, SEG // 2), :], BF16) for kc in range(FB)], axis=1)
                y = _dot(hrow, pltpu.bitcast(w2u[nb], BF16))
                ys[nb] = y + x_v[pl.ds(r0, SEG), pl.ds(nb * 128, 128)].astype(F32) + b2f[pl.ds(nb, 1), :]

            def do_q(h):
                if 0 <= h < H:
                    qs[h] = _dot(lhs, W(3 * h))

            def do_k(h):
                if 0 <= h < H:
                    ks[h] = _dot(lhs, W(3 * h + 1)).astype(BF16)

            def do_v(h):
                if 0 <= h < H:
                    vs_[h] = _dot(lhs, W(3 * h + 2)).astype(BF16)

            def do_qk(h):
                if 0 <= h < H:
                    sc = _dot(qs.pop(h), ks.pop(h), NT) * scale
                    sc = jnp.where(mask, sc, -1e9)
                    m = jnp.max(sc, axis=-1, keepdims=True)
                    e = jnp.exp(sc - m)
                    ls[h] = jnp.sum(e, axis=-1, keepdims=True)
                    es[h] = e

            def do_pv(h):
                if 0 <= h < H:
                    o = _dot(es.pop(h), vs_.pop(h)) / ls.pop(h)
                    o_buf[:, pl.ds(h * E, E)] = o

            if P2POS == 'a':
                pre, mid = [0, 1], {H - 1: [2], H: [3]}
                rest = [4, 5, 6, 7]
            elif P2POS == 'b':
                pre, mid = [0], {H - 1: [1], H: [2, 3]}
                rest = [4, 5, 6, 7]
            elif P2POS == 'c':
                pre, mid = [0, 1], {H - 2: [2], H - 1: [3], H: [4, 5]}
                rest = [6, 7]
            elif P2POS == 'd':
                pre, mid = [], {}
                rest = list(range(8))
            for nb in pre:
                do_y(nb)
            for i in range(-1, H + PVD):
                do_q(i + 1)
                do_qk(i)
                do_k(i + 1)
                do_v(i + 1)
                for nb in mid.get(i, []):
                    do_y(nb)
                do_pv(i - PVD)
            oall = o_buf[...]
            mems = []
            for nb in range(DB):
                if nb in rest:
                    do_y(nb)
                acc = _dot(oall, pltpu.bitcast(wou[nb], BF16))
                mems.append(acc[:MEM, :])
                out_v[pl.ds(r0, SEG), pl.ds(nb * 128, 128)] = (acc[MEM:, :] + ys.pop(nb)).astype(BF16)
            out_cp(s).start()
            return jnp.concatenate(mems, axis=1)

        def steps(i, mem):
            for u in range(UNR):
                mem = step(i * UNR + u, mem)
            return mem

        with _scope('CHAIN'):
            lax.fori_loop(0, NSEG // UNR, steps, mem0_ref[...].astype(F32))

        def drain(s, carry):
            out_cp(s).wait()
            return carry
        with _scope('DRAIN'):
            lax.fori_loop(0, NSEG, drain, 0)

    scratch = [
        pltpu.VMEM((S, D), BF16),
        pltpu.VMEM((S, D), F32),
        pltpu.VMEM((FB, S, 128), BF16),
        pltpu.VMEM((S, D), BF16),
        pltpu.VMEM((3, D, H, E), BF16),
        pltpu.VMEM((3 * H, D, E), BF16),
        pltpu.VMEM((DB, H * E, 128), BF16),
        pltpu.VMEM((FB, D, 128), BF16),
        pltpu.VMEM((DB, FF, 128), BF16),
        pltpu.VMEM((L, H * E), F32),
        pltpu.VMEM((FB, 128), F32),
        pltpu.VMEM((DB, 128), F32),
        pltpu.SemaphoreType.DMA((XCH,)),
        pltpu.SemaphoreType.DMA((FB,)),
        pltpu.SemaphoreType.DMA((DB,)),
        pltpu.SemaphoreType.DMA((DB,)),
        pltpu.SemaphoreType.DMA((3 * RCH,)),
        pltpu.SemaphoreType.DMA,
    ]
    anyspec = pl.BlockSpec(memory_space=pl.ANY)
    vspec = pl.BlockSpec(memory_space=pltpu.VMEM)
    return pl.pallas_call(
        kernel,
        out_shape=jax.ShapeDtypeStruct((S, D), BF16),
        in_specs=[anyspec, vspec, anyspec, anyspec, anyspec, anyspec, anyspec, vspec, anyspec, vspec],
        out_specs=anyspec,
        scratch_shapes=scratch,
        compiler_params=pltpu.CompilerParams(vmem_limit_bytes=126 * 1024 * 1024),
    )


@functools.partial(jax.jit, static_argnames=("A_seg_len",))
def pallas_parallel_sum__memory_aug_recurrent_mem_tr__dense_activation_gelu__prompt_kernel(A_x, A_mem0, A_Wq, A_Wk, A_Wv, A_Wo, A_seg_len, B_x, B_w1, B_b1, B_w2, B_b2):
    B, S, D = A_x.shape
    _, H, E = A_Wq.shape
    MEM = A_mem0.shape[1]
    FF = B_w1.shape[1]
    assert B == 1
    call = build(S, D, H, E, FF, MEM, int(A_seg_len))
    out = call(A_x.reshape(S, D), A_mem0.reshape(MEM, D), A_Wq, A_Wk, A_Wv, A_Wo.reshape(H * E, D),
               B_w1, B_b1.reshape(FF // 128, 128), B_w2, B_b2.reshape(D // 128, 128))
    return out.reshape(B, S, D)
```

```python
import functools

import jax
import jax.numpy as jnp
import numpy as np
from jax import lax
from jax.experimental import pallas as pl
from jax.experimental.pallas import tpu as pltpu

F32 = jnp.float32
BF16 = jnp.bfloat16
U32 = jnp.uint32

_NN = (((1,), (0,)), ((), ()))
_NT = (((1,), (1,)), ((), ()))
_LO16 = np.uint32(0xFFFF)
_HI16 = np.uint32(0xFFFF0000)


def _dot(a, b, dims=_NN):
    return lax.dot_general(a, b, dims, preferred_element_type=F32)


def _gelu_tanh(x):
    c = 0.7978845608028654
    return 0.5 * x * (1.0 + jnp.tanh(c * (x + 0.044715 * (x * x * x))))


def _transpose8(vs, sub):
    vs = list(vs)
    for dist in (4, 2, 1):
        keep = (sub & dist) == 0
        new = list(vs)
        for a in range(8):
            if a & dist:
                continue
            b = a + dist
            new[a] = jnp.where(keep, vs[a], pltpu.roll(vs[b], dist, 0))
            new[b] = jnp.where(keep, pltpu.roll(vs[a], 8 - dist, 0), vs[b])
        vs = new
    return vs


def _build(S, D, H, E, FF, MEM, SEG):
    L = MEM + SEG
    NSEG = S // SEG
    DB = D // 128
    FB = FF // 128
    XCH = 8
    XR = S // XCH
    PF = 4
    P1C = 2
    P1R = 256
    P1N = (FB - PF) // P1C
    RCH = 4
    RD = D // RCH
    UNR = 2
    OUTR = SEG * UNR
    QK_LAG, PV_LAG = 1, 3
    Y_PRE = (0, 1)
    Y_MID = {H - 3: 2, H - 2: 3, H - 1: 4, H: 5, H + 1: 6}
    Y_REST = (7,)
    scale = float(E) ** -0.5
    assert E == 128 and H % 16 == 0 and P1N == 3 * RCH and NSEG % UNR == 0
    assert XR % (PF * 16) == 0 and SEG % 16 == 0 and MEM % 8 == 0

    def kernel(x_hbm, mem0_ref, wq_hbm, wk_hbm, wv_hbm, wo_hbm, w1_hbm, b1_ref, w2_hbm, b2_ref,
               out_hbm,
               x_v, xn_v, h_v, out_v, stg, wqkv, wo_v, w1_v, w2_v, o_buf, b1_f, b2_f,
               sem_x, sem_w1, sem_w2, sem_wo, sem_stg, sem_out):
        w_hbm = (wq_hbm, wk_hbm, wv_hbm)

        def x_cp(c):
            return pltpu.make_async_copy(x_hbm.at[pl.ds(c * XR, XR), :],
                                         x_v.at[pl.ds(c * XR, XR), :], sem_x.at[c])

        def w1_cp(c):
            return pltpu.make_async_copy(w1_hbm.at[:, pl.ds(pl.multiple_of(c * 128, 128), 128)],
                                         w1_v.at[c], sem_w1.at[c])

        def w2_cp(c):
            return pltpu.make_async_copy(w2_hbm.at[:, pl.ds(c * 128, 128)], w2_v.at[c], sem_w2.at[c])

        def wo_cp(c):
            return pltpu.make_async_copy(wo_hbm.at[:, pl.ds(c * 128, 128)], wo_v.at[c], sem_wo.at[c])

        def stg_cp(k):
            t, c = divmod(k, RCH)
            return pltpu.make_async_copy(w_hbm[t].at[pl.ds(c * RD, RD)],
                                         stg.at[pl.ds(k * RD, RD)], sem_stg.at[k])

        def out_cp(i):
            r0 = pl.multiple_of(i * OUTR, OUTR)
            return pltpu.make_async_copy(out_v.at[pl.ds(r0, OUTR), :],
                                         out_hbm.at[pl.ds(r0, OUTR), :], sem_out)

        stg_u = stg.bitcast(U32)
        wqkv_u = wqkv.bitcast(U32)
        w1_u = w1_v.bitcast(U32)
        w2_u = w2_v.bitcast(U32)
        wo_u = wo_v.bitcast(U32)
        h_u = h_v.bitcast(U32)
        sub = lax.broadcasted_iota(jnp.int32, (8, 128), 0)

        def ln_rows(r0, n):
            xb = x_v[pl.ds(r0, n), :].astype(F32)
            xc = xb - jnp.mean(xb, axis=-1, keepdims=True)
            var = jnp.mean(xc * xc, axis=-1, keepdims=True)
            xn_v[pl.ds(r0, n), :] = xc * lax.rsqrt(var + 1e-5)

        def ffn1(c, r0, n):
            pre = _dot(xn_v[pl.ds(r0, n), :], pltpu.bitcast(w1_u[c], BF16)) + b1_f[pl.ds(c, 1), :]
            h_v[c, pl.ds(r0, n), :] = _gelu_tanh(pre).astype(BF16)
            return pre

        def relayout(it, g, pre):
            t = it // RCH
            d0 = pl.multiple_of(it * RD + g * 16, 16)
            o0 = pl.multiple_of((it % RCH) * (RD // 2) + g * 8, 8)
            tie = 0
            for half in range(H // 16):
                parity = []
                for p in range(2):
                    r = (tie * (P1R // 4)) % P1R
                    stg_u[3 * D, pl.ds(0, 8), :] = pltpu.bitcast(pre[r:r + 8, :], U32)
                    tie += 1
                    parity.append(_transpose8(
                        [stg_u[d0 + 2 * j + p, pl.ds(half * 8, 8), :] for j in range(8)], sub))
                even, odd = parity
                for s8 in range(8):
                    hp = half * 8 + s8
                    wqkv_u[6 * hp + t, pl.ds(o0, 8), :] = (even[s8] & _LO16) | (odd[s8] << 16)
                    wqkv_u[6 * hp + 3 + t, pl.ds(o0, 8), :] = (even[s8] >> 16) | (odd[s8] & _HI16)

        x_cp(0).start()
        for c in range(PF):
            w1_cp(c).start()
        x_cp(1).start()
        b1_f[...] = b1_ref[...].astype(F32)
        b2_f[...] = b2_ref[...].astype(F32)
        LNR = XR // PF
        x_cp(0).wait()
        x_cp(2).start()
        for j in range(PF):
            ln_rows(j * LNR, LNR)
        for c in range(PF):
            w1_cp(c).wait()

        for c in range(XCH):
            if c + 1 < XCH:
                x_cp(c + 1).wait()
            for j in range(PF):
                pre = ffn1(j, c * XR, XR)
                if j == 0:
                    if c + 3 < XCH:
                        x_cp(c + 3).start()
                    if c >= XCH - 3:
                        stg_cp(c - (XCH - 3)).start()
                    if c == XCH - 2:
                        for cb in range(PF, PF + 2 * P1C):
                            w1_cp(cb).start()
                if c + 1 < XCH:
                    x_v[pl.ds(S, 16), pl.ds(0, 128)] = pre[0:16, :].astype(BF16)
                    ln_rows((c + 1) * XR + j * LNR, LNR)

        def p1b(it, carry):
            for j in range(P1C):
                w1_cp(PF + it * P1C + j).wait()
            dst = stg.at[pl.ds(pl.multiple_of(it * RD, RD), RD)]
            pltpu.make_async_copy(dst, dst, sem_stg.at[it]).wait()
            nblk = P1C * (S // P1R)
            ng = RD // 16
            for bi in range(nblk):
                j, r = divmod(bi, S // P1R)
                pre = ffn1(PF + it * P1C + j, r * P1R, P1R)
                if bi == 0:
                    @pl.when(it + 2 < P1N)
                    def _():
                        for j2 in range(P1C):
                            w1_cp(PF + (it + 2) * P1C + j2).start()
                    for k in range(3, 3 * RCH):
                        @pl.when(it == k - 3)
                        def _(k=k):
                            stg_cp(k).start()
                    for c in range(DB):
                        @pl.when(it == 3 + c // 2)
                        def _(c=c):
                            wo_cp(c).start()

                        @pl.when(it == 5 + c // 2)
                        def _(c=c):
                            w2_cp(c).start()
                for g in range(bi * ng // nblk, (bi + 1) * ng // nblk):
                    relayout(it, g, pre)
            return carry

        lax.fori_loop(0, P1N, p1b, 0)
        for c in range(DB):
            wo_cp(c).wait()
            w2_cp(c).wait()

        qi = lax.broadcasted_iota(jnp.int32, (L, L), 0)
        ki = lax.broadcasted_iota(jnp.int32, (L, L), 1)
        mask = (qi < MEM) | (qi >= ki)

        def step(s, mem):
            r0 = pl.multiple_of(s * SEG, SEG)
            rh = pl.multiple_of(s * (SEG // 2), SEG // 2)
            lhs = jnp.concatenate([mem, xn_v[pl.ds(r0, SEG), :]], axis=0)
            q, k, v, e, den, y = {}, {}, {}, {}, {}, {}

            def proj(i):
                return _dot(lhs, pltpu.bitcast(wqkv_u[i], BF16))

            def ffn2(nb):
                hrow = jnp.concatenate(
                    [pltpu.bitcast(h_u[kc, pl.ds(rh, SEG // 2), :], BF16) for kc in range(FB)], axis=1)
                y[nb] = (_dot(hrow, pltpu.bitcast(w2_u[nb], BF16))
                         + x_v[pl.ds(r0, SEG), pl.ds(nb * 128, 128)].astype(F32)
                         + b2_f[pl.ds(nb, 1), :])

            def scores(h):
                sc = jnp.where(mask, _dot(q.pop(h), k.pop(h), _NT) * scale, -1e9)
                e[h] = jnp.exp(sc - jnp.max(sc, axis=-1, keepdims=True))
                den[h] = jnp.sum(e[h], axis=-1, keepdims=True)

            def context(h):
                o_buf[:, pl.ds(h * E, E)] = _dot(e.pop(h), v.pop(h)) / den.pop(h)

            for nb in Y_PRE:
                ffn2(nb)
            for i in range(H + PV_LAG):
                if i < H:
                    k[i] = proj(3 * i + 1).astype(BF16)
                    q[i] = proj(3 * i)
                if 0 <= i - QK_LAG < H:
                    scores(i - QK_LAG)
                if i < H:
                    v[i] = proj(3 * i + 2).astype(BF16)
                if i - QK_LAG in Y_MID:
                    ffn2(Y_MID[i - QK_LAG])
                if 0 <= i - PV_LAG < H:
                    context(i - PV_LAG)
            o_all = o_buf[...]
            mem_next = []
            for nb in range(DB):
                if nb in Y_REST:
                    ffn2(nb)
                acc = _dot(o_all, pltpu.bitcast(wo_u[nb], BF16))
                mem_next.append(acc[:MEM, :])
                out_v[pl.ds(r0, SEG), pl.ds(nb * 128, 128)] = (acc[MEM:, :] + y.pop(nb)).astype(BF16)
            return jnp.concatenate(mem_next, axis=1)

        def steps(i, mem):
            for u in range(UNR):
                mem = step(i * UNR + u, mem)
            out_cp(i).start()
            return mem

        lax.fori_loop(0, NSEG // UNR, steps, mem0_ref[...].astype(F32))

        def drain(i, carry):
            out_cp(i).wait()
            return carry

        lax.fori_loop(0, NSEG // UNR, drain, 0)

    scratch = [
        pltpu.VMEM((S + 16, D), BF16),
        pltpu.VMEM((S, D), F32),
        pltpu.VMEM((FB, S, 128), BF16),
        pltpu.VMEM((S, D), BF16),
        pltpu.VMEM((3 * D + 8, H, E), BF16),
        pltpu.VMEM((3 * H, D, E), BF16),
        pltpu.VMEM((DB, H * E, 128), BF16),
        pltpu.VMEM((FB, D, 128), BF16),
        pltpu.VMEM((DB, FF, 128), BF16),
        pltpu.VMEM((L, H * E), F32),
        pltpu.VMEM((FB, 128), F32),
        pltpu.VMEM((DB, 128), F32),
        pltpu.SemaphoreType.DMA((XCH,)),
        pltpu.SemaphoreType.DMA((FB,)),
        pltpu.SemaphoreType.DMA((DB,)),
        pltpu.SemaphoreType.DMA((DB,)),
        pltpu.SemaphoreType.DMA((3 * RCH,)),
        pltpu.SemaphoreType.DMA,
    ]
    hbm = pl.BlockSpec(memory_space=pl.ANY)
    vmem = pl.BlockSpec(memory_space=pltpu.VMEM)
    return pl.pallas_call(
        kernel,
        out_shape=jax.ShapeDtypeStruct((S, D), BF16),
        in_specs=[hbm, vmem, hbm, hbm, hbm, hbm, hbm, vmem, hbm, vmem],
        out_specs=hbm,
        scratch_shapes=scratch,
        compiler_params=pltpu.CompilerParams(vmem_limit_bytes=126 * 1024 * 1024),
    )


@functools.partial(jax.jit, static_argnames=("A_seg_len",))
def pallas_parallel_sum__memory_aug_recurrent_mem_tr__dense_activation_gelu__prompt_kernel(
    A_x, A_mem0, A_Wq, A_Wk, A_Wv, A_Wo, A_seg_len, B_x, B_w1, B_b1, B_w2, B_b2,
):
    del B_x
    B, S, D = A_x.shape
    _, H, E = A_Wq.shape
    MEM = A_mem0.shape[1]
    FF = B_w1.shape[1]
    assert B == 1
    call = _build(S, D, H, E, FF, MEM, int(A_seg_len))
    out = call(A_x.reshape(S, D), A_mem0.reshape(MEM, D), A_Wq, A_Wk, A_Wv, A_Wo.reshape(H * E, D),
               B_w1, B_b1.reshape(FF // 128, 128), B_w2, B_b2.reshape(D // 128, 128))
    return out.reshape(B, S, D)
```

```python
import functools

import jax
import jax.numpy as jnp
import numpy as np
from jax import lax
from jax.experimental import pallas as pl
from jax.experimental.pallas import tpu as pltpu

F32 = jnp.float32
BF16 = jnp.bfloat16
U32 = jnp.uint32

_NN = (((1,), (0,)), ((), ()))
_NT = (((1,), (1,)), ((), ()))
_LO16 = np.uint32(0xFFFF)
_HI16 = np.uint32(0xFFFF0000)


def _dot(a, b, dims=_NN):
    return lax.dot_general(a, b, dims, preferred_element_type=F32)


def _gelu_tanh(x):
    c = 0.7978845608028654
    return 0.5 * x * (1.0 + jnp.tanh(c * (x + 0.044715 * (x * x * x))))


def _transpose8(vs, sub):
    vs = list(vs)
    for dist in (4, 2, 1):
        keep = (sub & dist) == 0
        new = list(vs)
        for a in range(8):
            if a & dist:
                continue
            b = a + dist
            new[a] = jnp.where(keep, vs[a], pltpu.roll(vs[b], dist, 0))
            new[b] = jnp.where(keep, pltpu.roll(vs[a], 8 - dist, 0), vs[b])
        vs = new
    return vs


def _build(S, D, H, E, FF, MEM, SEG):
    L = MEM + SEG
    NSEG = S // SEG
    DB = D // 128
    FB = FF // 128
    XCH = 8
    XR = S // XCH
    PF = 4
    LNR = XR // PF
    XWAIT = {0: (1, 2), 2: (3, 4), 4: (5, 6, 7)}
    P1C = 4
    P1R = 256
    P1N = (FB - PF) // P1C
    RCH = 4
    RD = D // RCH
    CPI = 3 * RCH // P1N
    R2 = 2 * SEG
    QK_LAG, PV_LAG = 1, 3
    Y_SLOTS = (-1, H - 2 + QK_LAG, H + QK_LAG, H + 1 + QK_LAG)
    scale = float(E) ** -0.5
    assert E == 128 and H % 16 == 0 and NSEG % 2 == 0 and DB == 2 * len(Y_SLOTS)
    assert CPI * P1N == 3 * RCH and (FB - PF) % P1C == 0
    assert XR % (PF * 16) == 0 and SEG % 16 == 0 and MEM % 8 == 0

    def kernel(x_hbm, mem0_ref, wq_hbm, wk_hbm, wv_hbm, wo_hbm, w1_hbm, b1_ref, w2_hbm, b2_ref,
               out_hbm,
               x_v, xn_v, h_v, out_v, stg, wqkv, wo_v, w1_v, w2_v, o_buf, b1_f, b2_f,
               sem_x, sem_w1, sem_w2, sem_wo, sem_stg, sem_out):
        w_hbm = (wq_hbm, wk_hbm, wv_hbm)

        def x_cp(c):
            return pltpu.make_async_copy(x_hbm.at[pl.ds(c * XR, XR), :],
                                         x_v.at[pl.ds(c * XR, XR), :], sem_x.at[c])

        def w1_cp(c):
            return pltpu.make_async_copy(w1_hbm.at[:, pl.ds(pl.multiple_of(c * 128, 128), 128)],
                                         w1_v.at[c], sem_w1.at[c])

        def w2_cp(c):
            return pltpu.make_async_copy(w2_hbm.at[:, pl.ds(c * 128, 128)], w2_v.at[c], sem_w2.at[c])

        def wo_cp(c):
            return pltpu.make_async_copy(wo_hbm.at[:, pl.ds(c * 128, 128)], wo_v.at[c], sem_wo.at[c])

        def stg_cp(k):
            t, c = divmod(k, RCH)
            return pltpu.make_async_copy(w_hbm[t].at[pl.ds(c * RD, RD)],
                                         stg.at[pl.ds(k * RD, RD)], sem_stg.at[k])

        def out_cp(i):
            r0 = pl.multiple_of(i * R2, R2)
            return pltpu.make_async_copy(out_v.at[pl.ds(r0, R2), :],
                                         out_hbm.at[pl.ds(r0, R2), :], sem_out)

        stg_u = stg.bitcast(U32)
        wqkv_u = wqkv.bitcast(U32)
        w1_u = w1_v.bitcast(U32)
        w2_u = w2_v.bitcast(U32)
        wo_u = wo_v.bitcast(U32)
        h_u = h_v.bitcast(U32)
        sub = lax.broadcasted_iota(jnp.int32, (8, 128), 0)

        def ln_rows(r0, n):
            xb = x_v[pl.ds(r0, n), :].astype(F32)
            xc = xb - jnp.mean(xb, axis=-1, keepdims=True)
            var = jnp.mean(xc * xc, axis=-1, keepdims=True)
            xn_v[pl.ds(r0, n), :] = xc * lax.rsqrt(var + 1e-5)

        def ffn1(c, r0, n):
            pre = _dot(xn_v[pl.ds(r0, n), :], pltpu.bitcast(w1_u[c], BF16)) + b1_f[pl.ds(c, 1), :]
            h_v[c, pl.ds(r0, n), :] = _gelu_tanh(pre).astype(BF16)
            return pre

        def relayout(k, g, pre):
            t = k // RCH
            d0 = pl.multiple_of(k * RD + g * 16, 16)
            o0 = pl.multiple_of((k % RCH) * (RD // 2) + g * 8, 8)
            tie = 0
            for half in range(H // 16):
                parity = []
                for p in range(2):
                    r = (tie * (P1R // 4)) % P1R
                    stg_u[3 * D, pl.ds(0, 8), :] = pltpu.bitcast(pre[r:r + 8, :], U32)
                    tie += 1
                    parity.append(_transpose8(
                        [stg_u[d0 + 2 * j + p, pl.ds(half * 8, 8), :] for j in range(8)], sub))
                even, odd = parity
                for s8 in range(8):
                    hp = half * 8 + s8
                    wqkv_u[6 * hp + t, pl.ds(o0, 8), :] = (even[s8] & _LO16) | (odd[s8] << 16)
                    wqkv_u[6 * hp + 3 + t, pl.ds(o0, 8), :] = (even[s8] >> 16) | (odd[s8] & _HI16)

        x_cp(0).start()
        for c in range(PF):
            w1_cp(c).start()
        for c in range(1, XCH):
            x_cp(c).start()
        for c in range(PF, PF + P1C):
            w1_cp(c).start()
        for k in range(3 * RCH):
            stg_cp(k).start(priority=1)
        for c in range(DB):
            wo_cp(c).start(priority=1)
        for c in range(DB):
            w2_cp(c).start(priority=1)
        b1_f[...] = b1_ref[...].astype(F32)
        b2_f[...] = b2_ref[...].astype(F32)
        x_cp(0).wait()
        for j in range(PF):
            ln_rows(j * LNR, LNR)
        w1_cp(0).wait()

        for c in range(XCH):
            ties = ((2, 0), (2, XR // 2), (3, 0), (3, XR // 2)) if c == 0 else (
                (0, 0), (0, XR // 2), (1, 0), (1, XR // 2))
            for j in range(PF):
                if c == 0 and j > 0:
                    w1_cp(j).wait()
                pre = ffn1(j, c * XR, XR)
                if c + 1 == XCH:
                    continue
                for q, (tj, tr) in enumerate(ties):
                    if tj != j:
                        continue
                    if q == 0:
                        for cw in XWAIT.get(c, ()):
                            x_cp(cw).wait()
                    x_v[pl.ds(S, 16), pl.ds(0, 128)] = pre[tr:tr + 16, :].astype(BF16)
                    ln_rows((c + 1) * XR + q * LNR, LNR)

        def p1b(it, carry):
            for j in range(P1C):
                w1_cp(PF + it * P1C + j).wait()
            for q in range(CPI):
                dst = stg.at[pl.ds(pl.multiple_of((it * CPI + q) * RD, RD), RD)]
                pltpu.make_async_copy(dst, dst, sem_stg.at[it * CPI + q]).wait()
            nblk = P1C * (S // P1R)
            ng = RD // 16
            for bi in range(nblk):
                j, r = divmod(bi, S // P1R)
                pre = ffn1(PF + it * P1C + j, r * P1R, P1R)
                if bi == 0:
                    @pl.when(it + 1 < P1N)
                    def _():
                        for j2 in range(P1C):
                            w1_cp(PF + (it + 1) * P1C + j2).start()
                for g in range(bi * ng * CPI // nblk, (bi + 1) * ng * CPI // nblk):
                    relayout(it * CPI + g // ng, g % ng, pre)
            return carry

        lax.fori_loop(0, P1N, p1b, 0)
        for c in range(DB):
            wo_cp(c).wait()
            w2_cp(c).wait()

        qi = lax.broadcasted_iota(jnp.int32, (L, L), 0)
        ki = lax.broadcasted_iota(jnp.int32, (L, L), 1)
        mask = (qi < MEM) | (qi >= ki)

        def steps(i, mem):
            p0 = pl.multiple_of(i * R2, R2)
            ph = pl.multiple_of(i * SEG, SEG)
            y, pending = {}, {}

            def emit(u, nb, val):
                out_v[pl.ds(p0 + u * SEG, SEG), pl.ds(nb * 128, 128)] = val.astype(BF16)

            def ffn2(nb):
                hrow = jnp.concatenate(
                    [pltpu.bitcast(h_u[kc, pl.ds(ph, SEG), :], BF16) for kc in range(FB)], axis=1)
                y[nb] = (_dot(hrow, pltpu.bitcast(w2_u[nb], BF16))
                         + x_v[pl.ds(p0, R2), pl.ds(nb * 128, 128)].astype(F32)
                         + b2_f[pl.ds(nb, 1), :])
                if nb in pending:
                    emit(0, nb, pending.pop(nb) + y[nb][:SEG, :])

            for u in range(2):
                lhs = jnp.concatenate([mem, xn_v[pl.ds(p0 + u * SEG, SEG), :]], axis=0)
                q, k, v, e, den = {}, {}, {}, {}, {}

                def proj(n):
                    return _dot(lhs, pltpu.bitcast(wqkv_u[n], BF16))

                def scores(h):
                    sc = jnp.where(mask, _dot(q.pop(h), k.pop(h), _NT) * scale, -1e9)
                    e[h] = jnp.exp(sc - jnp.max(sc, axis=-1, keepdims=True))
                    den[h] = jnp.sum(e[h], axis=-1, keepdims=True)

                def context(h):
                    o_buf[:, pl.ds(h * E, E)] = _dot(e.pop(h), v.pop(h)) / den.pop(h)

                def filler(slot):
                    if slot in Y_SLOTS:
                        ffn2(u * len(Y_SLOTS) + Y_SLOTS.index(slot))

                filler(-1)
                for slot in range(H + PV_LAG):
                    if slot < H:
                        k[slot] = proj(3 * slot + 1).astype(BF16)
                        q[slot] = proj(3 * slot)
                    if 0 <= slot - QK_LAG < H:
                        scores(slot - QK_LAG)
                    if slot < H:
                        v[slot] = proj(3 * slot + 2).astype(BF16)
                    filler(slot)
                    if 0 <= slot - PV_LAG < H:
                        context(slot - PV_LAG)

                o_all = o_buf[...]
                mem_next = []
                for nb in range(DB):
                    acc = _dot(o_all, pltpu.bitcast(wo_u[nb], BF16))
                    mem_next.append(acc[:MEM, :])
                    if nb in y:
                        emit(u, nb, acc[MEM:, :] + y[nb][u * SEG:(u + 1) * SEG, :])
                    else:
                        pending[nb] = acc[MEM:, :]
                mem = jnp.concatenate(mem_next, axis=1)
            assert not pending and len(y) == DB
            out_cp(i).start()
            return mem

        lax.fori_loop(0, NSEG // 2, steps, mem0_ref[...].astype(F32))

        def drain(i, carry):
            out_cp(i).wait()
            return carry

        lax.fori_loop(0, NSEG // 2, drain, 0)

    scratch = [
        pltpu.VMEM((S + 16, D), BF16),
        pltpu.VMEM((S, D), F32),
        pltpu.VMEM((FB, S, 128), BF16),
        pltpu.VMEM((S, D), BF16),
        pltpu.VMEM((3 * D + 8, H, E), BF16),
        pltpu.VMEM((3 * H, D, E), BF16),
        pltpu.VMEM((DB, H * E, 128), BF16),
        pltpu.VMEM((FB, D, 128), BF16),
        pltpu.VMEM((DB, FF, 128), BF16),
        pltpu.VMEM((L, H * E), F32),
        pltpu.VMEM((FB, 128), F32),
        pltpu.VMEM((DB, 128), F32),
        pltpu.SemaphoreType.DMA((XCH,)),
        pltpu.SemaphoreType.DMA((FB,)),
        pltpu.SemaphoreType.DMA((DB,)),
        pltpu.SemaphoreType.DMA((DB,)),
        pltpu.SemaphoreType.DMA((3 * RCH,)),
        pltpu.SemaphoreType.DMA,
    ]
    hbm = pl.BlockSpec(memory_space=pl.ANY)
    vmem = pl.BlockSpec(memory_space=pltpu.VMEM)
    return pl.pallas_call(
        kernel,
        out_shape=jax.ShapeDtypeStruct((S, D), BF16),
        in_specs=[hbm, vmem, hbm, hbm, hbm, hbm, hbm, vmem, hbm, vmem],
        out_specs=hbm,
        scratch_shapes=scratch,
        compiler_params=pltpu.CompilerParams(vmem_limit_bytes=126 * 1024 * 1024),
    )


@functools.partial(jax.jit, static_argnames=("A_seg_len",))
def pallas_parallel_sum__memory_aug_recurrent_mem_tr__dense_activation_gelu__prompt_kernel(
    A_x, A_mem0, A_Wq, A_Wk, A_Wv, A_Wo, A_seg_len, B_x, B_w1, B_b1, B_w2, B_b2,
):
    del B_x
    B, S, D = A_x.shape
    _, H, E = A_Wq.shape
    MEM = A_mem0.shape[1]
    FF = B_w1.shape[1]
    assert B == 1
    call = _build(S, D, H, E, FF, MEM, int(A_seg_len))
    out = call(A_x.reshape(S, D), A_mem0.reshape(MEM, D), A_Wq, A_Wk, A_Wv, A_Wo.reshape(H * E, D),
               B_w1, B_b1.reshape(FF // 128, 128), B_w2, B_b2.reshape(D // 128, 128))
    return out.reshape(B, S, D)
```

```python
import functools

import jax
import jax.numpy as jnp
import numpy as np
from jax import lax
from jax.experimental import pallas as pl
from jax.experimental.pallas import tpu as pltpu

F32 = jnp.float32
BF16 = jnp.bfloat16
U32 = jnp.uint32

_NN = (((1,), (0,)), ((), ()))
_NT = (((1,), (1,)), ((), ()))
_LO16 = np.uint32(0xFFFF)
_HI16 = np.uint32(0xFFFF0000)


def _dot(a, b, dims=_NN):
    return lax.dot_general(a, b, dims, preferred_element_type=F32)


def _gelu_tanh(x):
    c = 0.7978845608028654
    return 0.5 * x * (1.0 + jnp.tanh(c * (x + 0.044715 * (x * x * x))))


def _transpose8(vs, sub):
    vs = list(vs)
    for dist in (4, 2, 1):
        keep = (sub & dist) == 0
        new = list(vs)
        for a in range(8):
            if a & dist:
                continue
            b = a + dist
            new[a] = jnp.where(keep, vs[a], pltpu.roll(vs[b], dist, 0))
            new[b] = jnp.where(keep, pltpu.roll(vs[a], 8 - dist, 0), vs[b])
        vs = new
    return vs


def _build(S, D, H, E, FF, MEM, SEG):
    L = MEM + SEG
    NSEG = S // SEG
    DB = D // 128
    FB = FF // 128
    XCH = 8
    XR = S // XCH
    PF = 4
    LNR = XR // PF
    XWAIT = {0: (1,), 1: (2,), 2: (3, 4), 4: (5, 6, 7)}
    T0 = ((2, 0), (2, XR // 2), (3, 0), (3, XR // 2))
    P1C = 4
    P1R = 256
    P1N = (FB - PF) // P1C
    RCH = 4
    RD = D // RCH
    CPI = 3 * RCH // P1N
    R2 = 2 * SEG
    QK_LAG, PV_LAG = 1, 3
    Y_SLOTS = (-1, H - 2 + QK_LAG, H + QK_LAG, H + 1 + QK_LAG)
    START = ('x0', 'b', 'w0', 'w1', 'w2', 'x1', 'w3', 'x2', 'x3', 'x4', 'x5', 'x6', 'x7',
             'w4', 'w5', 'w6', 'w7')
    scale = float(E) ** -0.5
    assert E == 128 and H % 16 == 0 and NSEG % 2 == 0 and DB == 2 * len(Y_SLOTS)
    assert CPI * P1N == 3 * RCH and (FB - PF) % P1C == 0
    assert XR % (PF * 16) == 0 and SEG % 16 == 0 and MEM % 8 == 0
    assert sorted(START) == sorted(
        ['b'] + ['x%d' % c for c in range(XCH)] + ['w%d' % c for c in range(PF + P1C)])
    assert sorted(c for v in XWAIT.values() for c in v) == list(range(1, XCH))
    assert all(any(c + 1 in XWAIT.get(c0, ()) for c0 in range(c + 1)) for c in range(XCH - 1))

    def kernel(x_hbm, mem0_hbm, wq_hbm, wk_hbm, wv_hbm, wo_hbm, w1_hbm, b1_hbm, w2_hbm, b2_hbm,
               out_hbm,
               x_v, xn_v, h_v, out_v, stg, wqkv, wo_v, w1_v, w2_v, o_buf, b1_f, b2_f,
               mem0_ref, b1_ref, b2_ref,
               sems, sem_out):
        o_x, o_w1, o_w2, o_wo, o_stg, o_sm = np.cumsum([0, XCH, FB, DB, DB, 3 * RCH]).tolist()
        w_hbm = (wq_hbm, wk_hbm, wv_hbm)

        def x_cp(c):
            return pltpu.make_async_copy(x_hbm.at[pl.ds(c * XR, XR), :],
                                         x_v.at[pl.ds(c * XR, XR), :], sems.at[o_x + c])

        def w1_cp(c):
            return pltpu.make_async_copy(w1_hbm.at[:, pl.ds(pl.multiple_of(c * 128, 128), 128)],
                                         w1_v.at[c], sems.at[o_w1 + c])

        def w2_cp(c):
            return pltpu.make_async_copy(w2_hbm.at[:, pl.ds(c * 128, 128)], w2_v.at[c], sems.at[o_w2 + c])

        def wo_cp(c):
            return pltpu.make_async_copy(wo_hbm.at[:, pl.ds(c * 128, 128)], wo_v.at[c], sems.at[o_wo + c])

        def stg_cp(k):
            t, c = divmod(k, RCH)
            return pltpu.make_async_copy(w_hbm[t].at[pl.ds(c * RD, RD)],
                                         stg.at[pl.ds(k * RD, RD)], sems.at[o_stg + k])

        def out_cp(i):
            r0 = pl.multiple_of(i * R2, R2)
            return pltpu.make_async_copy(out_v.at[pl.ds(r0, R2), :],
                                         out_hbm.at[pl.ds(r0, R2), :], sem_out)

        stg_u = stg.bitcast(U32)
        wqkv_u = wqkv.bitcast(U32)
        w1_u = w1_v.bitcast(U32)
        w2_u = w2_v.bitcast(U32)
        wo_u = wo_v.bitcast(U32)
        h_u = h_v.bitcast(U32)
        sub = lax.broadcasted_iota(jnp.int32, (8, 128), 0)

        def ln_rows(r0, n):
            xb = x_v[pl.ds(r0, n), :].astype(F32)
            xc = xb - jnp.mean(xb, axis=-1, keepdims=True)
            var = jnp.mean(xc * xc, axis=-1, keepdims=True)
            xn_v[pl.ds(r0, n), :] = xc * lax.rsqrt(var + 1e-5)

        def ffn1(c, r0, n):
            pre = _dot(xn_v[pl.ds(r0, n), :], pltpu.bitcast(w1_u[c], BF16)) + b1_f[pl.ds(c, 1), :]
            h_v[c, pl.ds(r0, n), :] = _gelu_tanh(pre).astype(BF16)
            return pre

        def relayout(k, g, pre):
            t = k // RCH
            d0 = pl.multiple_of(k * RD + g * 16, 16)
            o0 = pl.multiple_of((k % RCH) * (RD // 2) + g * 8, 8)
            tie = 0
            for half in range(H // 16):
                parity = []
                for p in range(2):
                    r = tie * (P1R // 8)
                    stg_u[3 * D, pl.ds(0, 8), :] = pltpu.bitcast(pre[r:r + 8, :], U32)
                    tie += 1
                    parity.append(_transpose8(
                        [stg_u[d0 + 2 * j + p, pl.ds(half * 8, 8), :] for j in range(8)], sub))
                even, odd = parity
                for s8 in range(8):
                    hp = half * 8 + s8
                    wqkv_u[6 * hp + t, pl.ds(o0, 8), :] = (even[s8] & _LO16) | (odd[s8] << 16)
                    wqkv_u[6 * hp + 3 + t, pl.ds(o0, 8), :] = (even[s8] >> 16) | (odd[s8] & _HI16)

        small = [pltpu.make_async_copy(b1_hbm, b1_ref, sems.at[o_sm + 0]),
                 pltpu.make_async_copy(b2_hbm, b2_ref, sems.at[o_sm + 1]),
                 pltpu.make_async_copy(mem0_hbm, mem0_ref, sems.at[o_sm + 2])]
        for tok in START:
            if tok == 'b':
                small[0].start()
            else:
                (x_cp if tok[0] == 'x' else w1_cp)(int(tok[1:])).start()
        small[1].start()
        small[2].start()
        for k in range(3 * RCH):
            stg_cp(k).start(priority=1)
        for c in range(DB):
            wo_cp(c).start(priority=1)
        for c in range(DB):
            w2_cp(c).start(priority=1)
        x_cp(0).wait()
        for j in range(PF):
            ln_rows(j * LNR, LNR)
        small[0].wait()
        b1_f[...] = b1_ref[...].astype(F32)
        w1_cp(0).wait()

        for c in range(XCH):
            ties = T0 if c == 0 else (
                (0, 0), (0, XR // 2), (1, 0), (1, XR // 2))
            for j in range(PF):
                if c == 0 and j > 0:
                    w1_cp(j).wait()
                pre = ffn1(j, c * XR, XR)
                if c + 1 == XCH:
                    continue
                for q, (tj, tr) in enumerate(ties):
                    if tj != j:
                        continue
                    if q == 0:
                        for cw in XWAIT.get(c, ()):
                            x_cp(cw).wait()
                    x_v[pl.ds(S, 16), pl.ds(0, 128)] = pre[tr:tr + 16, :].astype(BF16)
                    ln_rows((c + 1) * XR + q * LNR, LNR)

        def p1b(it, carry):
            for j in range(P1C):
                w1_cp(PF + it * P1C + j).wait()
            for q in range(CPI):
                dst = stg.at[pl.ds(pl.multiple_of((it * CPI + q) * RD, RD), RD)]
                pltpu.make_async_copy(dst, dst, sems.at[o_stg + it * CPI + q]).wait()
            nblk = P1C * (S // P1R)
            ng = RD // 16
            for bi in range(nblk):
                j, r = divmod(bi, S // P1R)
                pre = ffn1(PF + it * P1C + j, r * P1R, P1R)
                if bi == 0:
                    @pl.when(it + 1 < P1N)
                    def _():
                        for j2 in range(P1C):
                            w1_cp(PF + (it + 1) * P1C + j2).start()
                for g in range(bi * ng * CPI // nblk, (bi + 1) * ng * CPI // nblk):
                    relayout(it * CPI + g // ng, g % ng, pre)
            return carry

        lax.fori_loop(0, P1N, p1b, 0)
        for c in range(DB):
            wo_cp(c).wait()
            w2_cp(c).wait()
        small[1].wait()
        small[2].wait()
        b2_f[...] = b2_ref[...].astype(F32)

        qi = lax.broadcasted_iota(jnp.int32, (L, L), 0)
        ki = lax.broadcasted_iota(jnp.int32, (L, L), 1)
        mask = (qi < MEM) | (qi >= ki)

        def steps(i, mem):
            p0 = pl.multiple_of(i * R2, R2)
            ph = pl.multiple_of(i * SEG, SEG)
            y, pending = {}, {}

            def emit(u, nb, val):
                out_v[pl.ds(p0 + u * SEG, SEG), pl.ds(nb * 128, 128)] = val.astype(BF16)

            def ffn2(nb):
                hrow = jnp.concatenate(
                    [pltpu.bitcast(h_u[kc, pl.ds(ph, SEG), :], BF16) for kc in range(FB)], axis=1)
                y[nb] = (_dot(hrow, pltpu.bitcast(w2_u[nb], BF16))
                         + x_v[pl.ds(p0, R2), pl.ds(nb * 128, 128)].astype(F32)
                         + b2_f[pl.ds(nb, 1), :])
                if nb in pending:
                    emit(0, nb, pending.pop(nb) + y[nb][:SEG, :])

            for u in range(2):
                lhs = jnp.concatenate([mem, xn_v[pl.ds(p0 + u * SEG, SEG), :]], axis=0)
                q, k, v, e, den = {}, {}, {}, {}, {}

                def proj(n):
                    return _dot(lhs, pltpu.bitcast(wqkv_u[n], BF16))

                def scores(h):
                    sc = jnp.where(mask, _dot(q.pop(h), k.pop(h), _NT) * scale, -1e9)
                    e[h] = jnp.exp(sc - jnp.max(sc, axis=-1, keepdims=True))
                    den[h] = jnp.sum(e[h], axis=-1, keepdims=True)

                def context(h):
                    inv = pltpu.reciprocal(den.pop(h), approx=False, full_range=False)
                    o_buf[:, pl.ds(h * E, E)] = _dot(e.pop(h), v.pop(h)) * inv

                def filler(slot):
                    if slot in Y_SLOTS:
                        ffn2(u * len(Y_SLOTS) + Y_SLOTS.index(slot))

                filler(-1)
                for slot in range(H + PV_LAG):
                    if slot < H:
                        k[slot] = proj(3 * slot + 1).astype(BF16)
                        q[slot] = proj(3 * slot)
                    if 0 <= slot - QK_LAG < H:
                        scores(slot - QK_LAG)
                    if slot < H:
                        v[slot] = proj(3 * slot + 2).astype(BF16)
                    filler(slot)
                    if 0 <= slot - PV_LAG < H:
                        context(slot - PV_LAG)

                o_all = o_buf[...]
                mem_next = []
                for nb in range(DB):
                    acc = _dot(o_all, pltpu.bitcast(wo_u[nb], BF16))
                    mem_next.append(acc[:MEM, :])
                    if nb in y:
                        emit(u, nb, acc[MEM:, :] + y[nb][u * SEG:(u + 1) * SEG, :])
                    else:
                        pending[nb] = acc[MEM:, :]
                mem = jnp.concatenate(mem_next, axis=1)
            assert not pending and len(y) == DB
            out_cp(i).start()
            return mem

        lax.fori_loop(0, NSEG // 2, steps, mem0_ref[...].astype(F32))

        def drain(i, carry):
            out_cp(i).wait()
            return carry

        lax.fori_loop(0, NSEG // 2, drain, 0)

    scratch = [
        pltpu.VMEM((S + 16, D), BF16),
        pltpu.VMEM((S, D), F32),
        pltpu.VMEM((FB, S, 128), BF16),
        pltpu.VMEM((S, D), BF16),
        pltpu.VMEM((3 * D + 8, H, E), BF16),
        pltpu.VMEM((3 * H, D, E), BF16),
        pltpu.VMEM((DB, H * E, 128), BF16),
        pltpu.VMEM((FB, D, 128), BF16),
        pltpu.VMEM((DB, FF, 128), BF16),
        pltpu.VMEM((L, H * E), F32),
        pltpu.VMEM((FB, 128), F32),
        pltpu.VMEM((DB, 128), F32),
        pltpu.VMEM((MEM, D), BF16),
        pltpu.VMEM((FB, 128), BF16),
        pltpu.VMEM((DB, 128), BF16),
        pltpu.SemaphoreType.DMA((XCH + FB + 2 * DB + 3 * RCH + 3,)),
        pltpu.SemaphoreType.DMA,
    ]
    hbm = pl.BlockSpec(memory_space=pl.ANY)
    return pl.pallas_call(
        kernel,
        out_shape=jax.ShapeDtypeStruct((S, D), BF16),
        in_specs=[hbm] * 10,
        out_specs=hbm,
        scratch_shapes=scratch,
        compiler_params=pltpu.CompilerParams(vmem_limit_bytes=126 * 1024 * 1024),
    )


@functools.partial(jax.jit, static_argnames=("A_seg_len",))
def pallas_parallel_sum__memory_aug_recurrent_mem_tr__dense_activation_gelu__prompt_kernel(
    A_x, A_mem0, A_Wq, A_Wk, A_Wv, A_Wo, A_seg_len, B_x, B_w1, B_b1, B_w2, B_b2,
):
    del B_x
    B, S, D = A_x.shape
    _, H, E = A_Wq.shape
    MEM = A_mem0.shape[1]
    FF = B_w1.shape[1]
    assert B == 1
    call = _build(S, D, H, E, FF, MEM, int(A_seg_len))
    out = call(A_x.reshape(S, D), A_mem0.reshape(MEM, D), A_Wq, A_Wk, A_Wv, A_Wo.reshape(H * E, D),
               B_w1, B_b1.reshape(FF // 128, 128), B_w2, B_b2.reshape(D // 128, 128))
    return out.reshape(B, S, D)
```

```python
import functools

import jax
import jax.numpy as jnp
import numpy as np
from jax import lax
from jax.experimental import pallas as pl
from jax.experimental.pallas import tpu as pltpu

F32 = jnp.float32
BF16 = jnp.bfloat16
U32 = jnp.uint32

_NN = (((1,), (0,)), ((), ()))
_NT = (((1,), (1,)), ((), ()))
_LO16 = np.uint32(0xFFFF)
_HI16 = np.uint32(0xFFFF0000)


def _dot(a, b, dims=_NN):
    return lax.dot_general(a, b, dims, preferred_element_type=F32)


def _gelu_tanh(x):
    c = 0.7978845608028654
    return 0.5 * x * (1.0 + jnp.tanh(c * (x + 0.044715 * (x * x * x))))


def _transpose8(vs, sub):
    vs = list(vs)
    for dist in (4, 2, 1):
        keep = (sub & dist) == 0
        new = list(vs)
        for a in range(8):
            if a & dist:
                continue
            b = a + dist
            new[a] = jnp.where(keep, vs[a], pltpu.roll(vs[b], dist, 0))
            new[b] = jnp.where(keep, pltpu.roll(vs[a], 8 - dist, 0), vs[b])
        vs = new
    return vs


def _build(S, D, H, E, FF, MEM, SEG):
    L = MEM + SEG
    NSEG = S // SEG
    DB = D // 128
    FB = FF // 128
    XCH = 8
    XR = S // XCH
    PF = 4
    LNR = XR // PF
    XWAIT = {0: (1,), 1: (2,), 2: (3, 4), 4: (5, 6, 7)}
    LN_AT0, LN_AT = (2, 2, 3, 3), (0, 0, 1, 1)
    P1C = 4
    P1R = 256
    P1N = (FB - PF) // P1C
    RCH = 4
    RD = D // RCH
    CPI = 3 * RCH // P1N
    R2 = 2 * SEG
    QK_LAG, PV_LAG = 1, 3
    Y_SLOTS = (-1, H - 2 + QK_LAG, H + QK_LAG, H + 1 + QK_LAG)
    START = ('x0', 'b', 'w0', 'w1', 'w2', 'x1', 'w3', 'x2', 'x3', 'x4', 'x5', 'x6', 'x7',
             'w4', 'w5', 'w6', 'w7')
    scale = float(E) ** -0.5
    assert E == 128 and H % 16 == 0 and NSEG % 2 == 0 and DB == 2 * len(Y_SLOTS)
    assert CPI * P1N == 3 * RCH and (FB - PF) % P1C == 0
    assert XR % (PF * 16) == 0 and SEG % 16 == 0 and MEM % 8 == 0
    assert sorted(START) == sorted(
        ['b'] + ['x%d' % c for c in range(XCH)] + ['w%d' % c for c in range(PF + P1C)])
    assert len(LN_AT0) == len(LN_AT) == PF
    assert sorted(c for v in XWAIT.values() for c in v) == list(range(1, XCH))
    assert all(any(c + 1 in XWAIT.get(c0, ()) for c0 in range(c + 1)) for c in range(XCH - 1))

    def kernel(x_hbm, mem0_hbm, wq_hbm, wk_hbm, wv_hbm, wo_hbm, w1_hbm, b1_hbm, w2_hbm, b2_hbm,
               out_hbm,
               x_v, xn_v, h_v, out_v, stg, wqkv, wo_v, w1_v, w2_v, o_buf, b1_f, b2_f,
               mem0_ref, b1_ref, b2_ref,
               sems, sem_out):
        o_x, o_w1, o_w2, o_wo, o_stg, o_sm = np.cumsum([0, XCH, FB, DB, DB, 3 * RCH]).tolist()
        w_hbm = (wq_hbm, wk_hbm, wv_hbm)

        def x_cp(c):
            return pltpu.make_async_copy(x_hbm.at[pl.ds(c * XR, XR), :],
                                         x_v.at[pl.ds(c * XR, XR), :], sems.at[o_x + c])

        def w1_cp(c):
            return pltpu.make_async_copy(w1_hbm.at[:, pl.ds(pl.multiple_of(c * 128, 128), 128)],
                                         w1_v.at[c], sems.at[o_w1 + c])

        def w2_cp(c):
            return pltpu.make_async_copy(w2_hbm.at[:, pl.ds(c * 128, 128)], w2_v.at[c], sems.at[o_w2 + c])

        def wo_cp(c):
            return pltpu.make_async_copy(wo_hbm.at[:, pl.ds(c * 128, 128)], wo_v.at[c], sems.at[o_wo + c])

        def stg_cp(k):
            t, c = divmod(k, RCH)
            return pltpu.make_async_copy(w_hbm[t].at[pl.ds(c * RD, RD)],
                                         stg.at[pl.ds(k * RD, RD)], sems.at[o_stg + k])

        def out_cp(i):
            r0 = pl.multiple_of(i * R2, R2)
            return pltpu.make_async_copy(out_v.at[pl.ds(r0, R2), :],
                                         out_hbm.at[pl.ds(r0, R2), :], sem_out)

        stg_u = stg.bitcast(U32)
        wqkv_u = wqkv.bitcast(U32)
        w1_u = w1_v.bitcast(U32)
        w2_u = w2_v.bitcast(U32)
        wo_u = wo_v.bitcast(U32)
        h_u = h_v.bitcast(U32)
        sub = lax.broadcasted_iota(jnp.int32, (8, 128), 0)

        def ln_rows(r0, n):
            xb = x_v[pl.ds(r0, n), :].astype(F32)
            xc = xb - jnp.mean(xb, axis=-1, keepdims=True)
            var = jnp.mean(xc * xc, axis=-1, keepdims=True)
            xn_v[pl.ds(r0, n), :] = xc * lax.rsqrt(var + 1e-5)

        def ffn1(c, r0, n):
            pre = _dot(xn_v[pl.ds(r0, n), :], pltpu.bitcast(w1_u[c], BF16)) + b1_f[pl.ds(c, 1), :]
            h_v[c, pl.ds(r0, n), :] = _gelu_tanh(pre).astype(BF16)
            return pre

        def relayout(k, g, pre):
            t = k // RCH
            d0 = pl.multiple_of(k * RD + g * 16, 16)
            o0 = pl.multiple_of((k % RCH) * (RD // 2) + g * 8, 8)
            tie = 0
            for half in range(H // 16):
                parity = []
                for p in range(2):
                    r = tie * (P1R // 8)
                    stg_u[3 * D, pl.ds(0, 8), :] = pltpu.bitcast(pre[r:r + 8, :], U32)
                    tie += 1
                    parity.append(_transpose8(
                        [stg_u[d0 + 2 * j + p, pl.ds(half * 8, 8), :] for j in range(8)], sub))
                even, odd = parity
                for s8 in range(8):
                    hp = half * 8 + s8
                    wqkv_u[6 * hp + t, pl.ds(o0, 8), :] = (even[s8] & _LO16) | (odd[s8] << 16)
                    wqkv_u[6 * hp + 3 + t, pl.ds(o0, 8), :] = (even[s8] >> 16) | (odd[s8] & _HI16)

        small = [pltpu.make_async_copy(b1_hbm, b1_ref, sems.at[o_sm + 0]),
                 pltpu.make_async_copy(b2_hbm, b2_ref, sems.at[o_sm + 1]),
                 pltpu.make_async_copy(mem0_hbm, mem0_ref, sems.at[o_sm + 2])]
        for tok in START:
            if tok == 'b':
                small[0].start()
            else:
                (x_cp if tok[0] == 'x' else w1_cp)(int(tok[1:])).start()
        small[1].start()
        small[2].start()
        for it in range(P1N):
            if it > 0:
                for j in range(P1C):
                    w1_cp(PF + it * P1C + j).start(priority=1)
            for q in range(CPI):
                stg_cp(it * CPI + q).start(priority=1)
        for c in range(DB):
            wo_cp(c).start(priority=1)
        for c in range(DB):
            w2_cp(c).start(priority=1)
        x_cp(0).wait()
        for j in range(PF):
            ln_rows(j * LNR, LNR)
        small[0].wait()
        b1_f[...] = b1_ref[...].astype(F32)
        w1_cp(0).wait()

        for c in range(XCH):
            at = LN_AT0 if c == 0 else LN_AT
            for j in range(PF):
                if c == 0 and j > 0:
                    w1_cp(j).wait()
                ffn1(j, c * XR, XR)
                if c + 1 == XCH:
                    continue
                if j == at[0]:
                    for cw in XWAIT.get(c, ()):
                        x_cp(cw).wait()
                for q in range(PF):
                    if at[q] == j:
                        ln_rows((c + 1) * XR + q * LNR, LNR)

        def p1b(it, carry):
            for j in range(P1C):
                w1_cp(PF + it * P1C + j).wait()
            for q in range(CPI):
                dst = stg.at[pl.ds(pl.multiple_of((it * CPI + q) * RD, RD), RD)]
                pltpu.make_async_copy(dst, dst, sems.at[o_stg + it * CPI + q]).wait()
            nblk = P1C * (S // P1R)
            ng = RD // 16
            for bi in range(nblk):
                j, r = divmod(bi, S // P1R)
                pre = ffn1(PF + it * P1C + j, r * P1R, P1R)
                for g in range(bi * ng * CPI // nblk, (bi + 1) * ng * CPI // nblk):
                    relayout(it * CPI + g // ng, g % ng, pre)
            return carry

        lax.fori_loop(0, P1N, p1b, 0)
        for c in range(DB):
            wo_cp(c).wait()
            w2_cp(c).wait()
        small[1].wait()
        small[2].wait()
        b2_f[...] = b2_ref[...].astype(F32)

        qi = lax.broadcasted_iota(jnp.int32, (L, L), 0)
        ki = lax.broadcasted_iota(jnp.int32, (L, L), 1)
        mask = (qi < MEM) | (qi >= ki)

        def steps(i, mem):
            p0 = pl.multiple_of(i * R2, R2)
            ph = pl.multiple_of(i * SEG, SEG)
            y, pending = {}, {}

            def emit(u, nb, val):
                out_v[pl.ds(p0 + u * SEG, SEG), pl.ds(nb * 128, 128)] = val.astype(BF16)

            def ffn2(nb):
                hrow = jnp.concatenate(
                    [pltpu.bitcast(h_u[kc, pl.ds(ph, SEG), :], BF16) for kc in range(FB)], axis=1)
                y[nb] = (_dot(hrow, pltpu.bitcast(w2_u[nb], BF16))
                         + x_v[pl.ds(p0, R2), pl.ds(nb * 128, 128)].astype(F32)
                         + b2_f[pl.ds(nb, 1), :])
                if nb in pending:
                    emit(0, nb, pending.pop(nb) + y[nb][:SEG, :])

            for u in range(2):
                lhs = jnp.concatenate([mem, xn_v[pl.ds(p0 + u * SEG, SEG), :]], axis=0)
                q, k, v, e, den = {}, {}, {}, {}, {}

                def proj(n):
                    return _dot(lhs, pltpu.bitcast(wqkv_u[n], BF16))

                def scores(h):
                    sc = jnp.where(mask, _dot(q.pop(h), k.pop(h), _NT) * scale, -1e9)
                    e[h] = jnp.exp(sc - jnp.max(sc, axis=-1, keepdims=True))
                    den[h] = jnp.sum(e[h], axis=-1, keepdims=True)

                def context(h):
                    inv = pltpu.reciprocal(den.pop(h), approx=False, full_range=False)
                    o_buf[:, pl.ds(h * E, E)] = _dot(e.pop(h), v.pop(h)) * inv

                def filler(slot):
                    if slot in Y_SLOTS:
                        ffn2(u * len(Y_SLOTS) + Y_SLOTS.index(slot))

                filler(-1)
                for slot in range(H + PV_LAG):
                    if slot < H:
                        k[slot] = proj(3 * slot + 1).astype(BF16)
                        q[slot] = proj(3 * slot)
                    if 0 <= slot - QK_LAG < H:
                        scores(slot - QK_LAG)
                    if slot < H:
                        v[slot] = proj(3 * slot + 2).astype(BF16)
                    filler(slot)
                    if 0 <= slot - PV_LAG < H:
                        context(slot - PV_LAG)

                o_all = o_buf[...]
                mem_next = []
                for nb in range(DB):
                    acc = _dot(o_all, pltpu.bitcast(wo_u[nb], BF16))
                    mem_next.append(acc[:MEM, :])
                    if nb in y:
                        emit(u, nb, acc[MEM:, :] + y[nb][u * SEG:(u + 1) * SEG, :])
                    else:
                        pending[nb] = acc[MEM:, :]
                mem = jnp.concatenate(mem_next, axis=1)
            assert not pending and len(y) == DB
            out_cp(i).start()
            return mem

        lax.fori_loop(0, NSEG // 2, steps, mem0_ref[...].astype(F32))

        def drain(i, carry):
            out_cp(i).wait()
            return carry

        lax.fori_loop(0, NSEG // 2, drain, 0)

    scratch = [
        pltpu.VMEM((S, D), BF16),
        pltpu.VMEM((S, D), F32),
        pltpu.VMEM((FB, S, 128), BF16),
        pltpu.VMEM((S, D), BF16),
        pltpu.VMEM((3 * D + 8, H, E), BF16),
        pltpu.VMEM((3 * H, D, E), BF16),
        pltpu.VMEM((DB, H * E, 128), BF16),
        pltpu.VMEM((FB, D, 128), BF16),
        pltpu.VMEM((DB, FF, 128), BF16),
        pltpu.VMEM((L, H * E), F32),
        pltpu.VMEM((FB, 128), F32),
        pltpu.VMEM((DB, 128), F32),
        pltpu.VMEM((MEM, D), BF16),
        pltpu.VMEM((FB, 128), BF16),
        pltpu.VMEM((DB, 128), BF16),
        pltpu.SemaphoreType.DMA((XCH + FB + 2 * DB + 3 * RCH + 3,)),
        pltpu.SemaphoreType.DMA,
    ]
    hbm = pl.BlockSpec(memory_space=pl.ANY)
    return pl.pallas_call(
        kernel,
        out_shape=jax.ShapeDtypeStruct((S, D), BF16),
        in_specs=[hbm] * 10,
        out_specs=hbm,
        scratch_shapes=scratch,
        compiler_params=pltpu.CompilerParams(vmem_limit_bytes=126 * 1024 * 1024),
    )


@functools.partial(jax.jit, static_argnames=("A_seg_len",))
def pallas_parallel_sum__memory_aug_recurrent_mem_tr__dense_activation_gelu__prompt_kernel(
    A_x, A_mem0, A_Wq, A_Wk, A_Wv, A_Wo, A_seg_len, B_x, B_w1, B_b1, B_w2, B_b2,
):
    del B_x
    B, S, D = A_x.shape
    _, H, E = A_Wq.shape
    MEM = A_mem0.shape[1]
    FF = B_w1.shape[1]
    assert B == 1
    call = _build(S, D, H, E, FF, MEM, int(A_seg_len))
    out = call(A_x.reshape(S, D), A_mem0.reshape(MEM, D), A_Wq, A_Wk, A_Wv, A_Wo.reshape(H * E, D),
               B_w1, B_b1.reshape(FF // 128, 128), B_w2, B_b2.reshape(D // 128, 128))
    return out.reshape(B, S, D)
```
